```python
import os as _os
_os.environ.setdefault("JAX_PLATFORMS", "cpu")
import jax
import jax.numpy as jnp

def _softmax(x, axis=-1):
    return jax.nn.softmax(x, axis=axis)
def _gelu(x):
    return jax.nn.gelu(x, approximate=True)
def _silu(x):
    return jax.nn.silu(x)
def _sigmoid(x):
    return jax.nn.sigmoid(x)
def _layernorm(x, axis=-1, eps=1e-5):
    m = jnp.mean(x, axis=axis, keepdims=True)
    v = jnp.var(x, axis=axis, keepdims=True)
    return (x - m) / jnp.sqrt(v + eps)
def _scatter_add(tgt, idx, src, axis=0):
    return tgt.at[idx].add(src)
def _segment_sum(src, seg, n):
    return jax.ops.segment_sum(src, seg, n)
class _Rng:
    def __init__(self, key):
        self._k = key
    def _next(self):
        self._k, sub = jax.random.split(self._k)
        return sub
    def normal(self, shape):
        return jax.random.normal(self._next(), shape, dtype=jnp.bfloat16)
    def randint(self, lo, hi, shape):
        return jax.random.randint(self._next(), shape, lo, hi, dtype=jnp.int32)
    def uniform(self, shape, lo=0.0, hi=1.0):
        return jax.random.uniform(self._next(), shape, jnp.bfloat16, lo, hi)
    def permutation(self, n):
        return jax.random.permutation(self._next(), n)


kernel_name = 'parallel_sum__softmax_full_mha__moe_arch_mod__prompt'

def setup_inputs():
    _rng = _Rng(jax.random.key(int.from_bytes(__import__("os").urandom(4), "little")))
    _w = (lambda a: (lambda t: t.astype(jnp.bfloat16) if jnp.issubdtype(t.dtype, jnp.floating) else t)(jnp.asarray(a)))
    def _A_setup():
        B, S, D = 1, 2048, 512
        return {
            "x": _w((lambda *s: _rng.normal(s) * 0.05)(B, S, D)),
            "wqkv": _w((lambda *s: _rng.normal(s) * 0.1)(D, 3 * D)),
            "wo": _w((lambda *s: _rng.normal(s) * 0.05)(D, D)),
        }
    _A_in = _A_setup()

    def _B_setup():
        B, S, D, F, C = 1, 2048, 512, 1792, 1
        return {
            "x": _w((lambda *s: _rng.normal(s) * 0.05)(B, S, D)),
            "w_r": _w((lambda *s: _rng.normal(s) * 1.6)(D)),
            "w_gate": _w((lambda *s: _rng.normal(s) * 0.1)(D, F)),
            "w_up": _w((lambda *s: _rng.normal(s) * 0.1)(D, F)),
            "w_down": _w((lambda *s: _rng.normal(s) * 0.1)(F, D)),
        }
    _B_in = _B_setup()

    return {
        "A_x": _A_in["x"],
        "A_wqkv": _A_in["wqkv"],
        "A_wo": _A_in["wo"],
        "B_x": _B_in["x"],
        "B_w_r": _B_in["w_r"],
        "B_w_gate": _B_in["w_gate"],
        "B_w_up": _B_in["w_up"],
        "B_w_down": _B_in["w_down"],
    }

def reference(A_x, A_wqkv, A_wo, B_x, B_w_r, B_w_gate, B_w_up, B_w_down):
    def _A_ref(x, wqkv, wo):
        B, S, D = x.shape
        H = 32; Dh = D // H
        qkv = (lambda x, *d: x.transpose(*d))((x @ wqkv).reshape(B, S, 3, H, Dh), 2, 0, 3, 1, 4)
        q, k, v = qkv[0], qkv[1], qkv[2]
        scale = Dh ** -0.5
        scores = jnp.einsum("bhqd,bhkd->bhqk", q, k) * scale
        p = _softmax(scores, axis=-1)
        o = jnp.einsum("bhqk,bhkd->bhqd", p, v)
        return (lambda x, *d: x.transpose(*d))(o, 0, 2, 1, 3).reshape(B, S, D) @ wo

    def _B_ref(x, w_r, w_gate, w_up, w_down):
        B, S, D = x.shape
        C = 1
        r = x @ w_r
        idx = jnp.argsort(-r, axis=-1)[:, :C]
        idx_e = jnp.repeat(idx.reshape(B, C, 1), D, axis=2)
        x_sel = jnp.take_along_axis(x, idx_e, axis=1)
        g = _silu(x_sel @ w_gate)
        u = x_sel @ w_up
        y = (g * u) @ w_down
        r_sel = _sigmoid(jnp.take_along_axis(r, idx, axis=1))
        y = y * r_sel.reshape(B, C, 1)
        b_off = (jnp.arange(B) * S).reshape(B, 1)
        flat_idx = (idx + b_off).reshape(B * C)
        zero = (x * 0.0).reshape(B * S, D)
        upd = _scatter_add(zero, flat_idx, y.reshape(B * C, D), axis=0)
        return x + upd.reshape(B, S, D)

    x = A_x
    xn = _layernorm(x, axis=-1)
    return x + _A_ref(xn, A_wqkv, A_wo) + _B_ref(xn, B_w_r, B_w_gate, B_w_up, B_w_down)
```

```python
import functools
import math

import jax
import jax.numpy as jnp
import jax.experimental.pallas as pl
import jax.experimental.pallas.tpu as pltpu

_H = 32
_DH = 16
_HG = 8
_BQ = 512
_R = 128
_UNROLL = 4
_TB = 512
_EPS = 1e-5
_L_LO = 2.0 ** -80
_L_HI = 2.0 ** 90

_f32 = jnp.float32
_bf16 = jnp.bfloat16


def _as_bf16(u):
    return pltpu.bitcast(u, _bf16)


def _as_u32(x):
    return pltpu.bitcast(x, jnp.uint32)


def _rnd(x):
    return x.astype(_bf16).astype(_f32)


def _kernel(x_hbm, wqkv_hbm, wo_hbm, wr_hbm, wg_hbm, wu_hbm, wd_hbm, out_hbm,
            x_v, wqkv_v, wo_v, wr_v, wg_v, wu_v, wd_v,
            xn_v, wt_v, k_v, qt_v, vt_v, r_v, p0, p1, qm0, qm1, ot_v, bad_v,
            upd_v, idx_s, out_v, sem_x, sem_w, sem_o):
    S, D = x_v.shape
    F = wg_v.shape[1]
    ntb = S // _TB
    nqb = S // _BQ
    nitems = _H * nqb
    nchunks = S // _R
    qscale = (_DH ** -0.5) * math.log2(math.e)

    def x_copy(b):
        return pltpu.make_async_copy(
            x_hbm.at[0, pl.ds(b * _TB, _TB), :], x_v.at[pl.ds(b * _TB, _TB), :], sem_x.at[b])

    w_copies = [
        pltpu.make_async_copy(wqkv_hbm, wqkv_v, sem_w.at[0]),
        pltpu.make_async_copy(wr_hbm, wr_v, sem_w.at[1]),
        pltpu.make_async_copy(wg_hbm, wg_v, sem_w.at[2]),
        pltpu.make_async_copy(wu_hbm, wu_v, sem_w.at[3]),
        pltpu.make_async_copy(wd_hbm, wd_v, sem_w.at[4]),
        pltpu.make_async_copy(wo_hbm, wo_v, sem_w.at[5]),
    ]
    c_qkv, c_r, c_g, c_u, c_d, c_o = w_copies
    c_qkv.start()
    c_r.start()
    for b in range(ntb):
        x_copy(b).start()
    c_g.start()
    c_u.start()
    c_d.start()
    c_o.start()

    c_qkv.wait()
    c_r.wait()
    wt_v[pl.ds(0, D), :] = wqkv_v[:, pl.ds(0, D)].T
    wt_v[pl.ds(D, D), :] = wqkv_v[:, pl.ds(2 * D, D)].T
    wt_v[pl.ds(2 * D, 16), :] = jnp.broadcast_to(wr_v[...].reshape(1, D), (16, D))

    eps_b = _rnd(jnp.full((1, 1), _EPS, _f32))
    for b in range(ntb):
        rows = pl.ds(b * _TB, _TB)
        x_copy(b).wait()
        xb = x_v[rows, :].astype(_f32)
        mean = jnp.mean(xb, axis=-1, keepdims=True)
        var = jnp.mean(jnp.square(xb - mean), axis=-1, keepdims=True)
        cen = _rnd(xb - _rnd(mean))
        den = _rnd(jnp.sqrt(_rnd(_rnd(var) + eps_b)))
        xn = (cen / den).astype(_bf16)
        xn_v[rows, :] = xn
        kk = jnp.dot(xn, wqkv_v[:, pl.ds(D, D)], preferred_element_type=_f32).astype(_bf16)
        for g in range(D // 128):
            k_v[g, pl.ds(b * _TB // 2, _TB // 2), :] = _as_u32(kk[:, g * 128:(g + 1) * 128])
        tt = jax.lax.dot_general(wt_v[...], xn, (((1,), (1,)), ((), ())),
                                 preferred_element_type=_f32)
        qt_v[:, rows] = _as_u32((tt[:D] * qscale).astype(_bf16))
        vt_v[:, rows] = _as_u32(tt[D:2 * D].astype(_bf16))
        r_v[:, rows] = tt[2 * D:2 * D + 8]

    r = _rnd(r_v[pl.ds(0, 1), :])
    rmax = jnp.max(r, axis=1, keepdims=True)
    pos = jax.lax.broadcasted_iota(jnp.int32, (1, S), 1)
    idx = jnp.min(jnp.where(r == rmax, pos, S - 1))
    idx_s[0] = idx
    base = pl.multiple_of((idx // 16) * 16, 16)
    grp = xn_v[pl.ds(base, 16), :].astype(_f32)
    sel = jax.lax.broadcasted_iota(jnp.int32, (16, D), 0) == (idx - base)
    x_sel = jnp.sum(jnp.where(sel, grp, 0.0), axis=0, keepdims=True)
    x_sel = jnp.broadcast_to(x_sel, (16, D)).astype(_bf16)
    c_g.wait()
    c_u.wait()
    c_d.wait()
    ga = _rnd(jnp.dot(x_sel, wg_v[...], preferred_element_type=_f32))
    ua = _rnd(jnp.dot(x_sel, wu_v[...], preferred_element_type=_f32))
    act = _rnd(ga * _rnd(jax.nn.sigmoid(ga)))
    hh = (act * ua).astype(_bf16)
    y = _rnd(jnp.dot(hh, wd_v[...], preferred_element_type=_f32))
    gate = _rnd(jax.nn.sigmoid(rmax))
    upd_v[...] = _rnd(y[:8] * gate)

    def split(item):
        item = jnp.clip(item, 0, nitems - 1)
        return item % _H, item // _H

    def prep(item, qm):
        h, qb = split(item)
        g = h // _HG
        q = qt_v[pl.ds(pl.multiple_of(g * 64, 64), 64), pl.ds(pl.multiple_of(qb * _BQ, _BQ), _BQ)]
        hrow = jax.lax.broadcasted_iota(jnp.int32, (64, _BQ), 0) // 8
        qm[...] = jnp.where(hrow == h % _HG, q, jnp.uint32(0))

    def step(item, do_a, pa, qm, qm_next, pb, lb, bad):
        g = split(item)[0] // _HG
        hb, qbb = split(item - 1)
        vrow = pl.ds(pl.multiple_of(hb * 8, 8), 8)
        l = jnp.zeros((8, _BQ), _f32)
        acc = jnp.zeros((16, _BQ), _f32)
        for c in range(nchunks):
            half = pl.ds(c * _R // 2, _R // 2)
            if do_a:
                st = jnp.dot(_as_bf16(k_v[g, half, :]), _as_bf16(qm[...]),
                             preferred_element_type=_f32)
                p = jnp.exp2(st)
                pa[half, :] = _as_u32(p.astype(_bf16))
                l = l + jnp.sum(p.reshape(_R // 8, 8, _BQ), axis=0)
                if c == nchunks // 2:
                    prep(item + 1, qm_next)
            acc = acc + jnp.dot(_as_bf16(vt_v[vrow, pl.ds(c * _R, _R)]), _as_bf16(pb[half, :]),
                                preferred_element_type=_f32)
        o = acc / lb
        ot_v[vrow, pl.ds(pl.multiple_of(qbb * _BQ, _BQ), _BQ)] = _as_u32(o.astype(_bf16))
        ok = (lb >= _L_LO) & (lb <= _L_HI)
        fin = (jnp.abs(o[:8]) < jnp.inf) & (jnp.abs(o[8:]) < jnp.inf)
        bad = jnp.where(ok & fin, bad, 1.0)
        return jnp.sum(l, axis=0, keepdims=True), bad

    p1[...] = jnp.zeros(p1.shape, jnp.uint32)
    prep(0, qm0)

    def body(j, carry):
        l1, bad = carry
        for u in range(0, _UNROLL, 2):
            it = j * _UNROLL + u
            l0, bad = step(it, True, p0, qm0, qm1, p1, l1, bad)
            l1, bad = step(it + 1, True, p1, qm1, qm0, p0, l0, bad)
        return l1, bad

    l1, bad = jax.lax.fori_loop(
        0, nitems // _UNROLL, body,
        (jnp.ones((1, _BQ), _f32), jnp.zeros((8, _BQ), _f32)))
    _, bad = step(nitems, False, None, None, None, p1, l1, bad)

    @pl.when(jnp.max(bad) > 0.0)
    def _():
        rc = 512

        def item_body(item, _):
            h, qb = split(item)
            g = h // _HG
            prep(item, qm0)
            vrow = pl.ds(pl.multiple_of(h * 8, 8), 8)

            def chunk(c, carry):
                m, l, acc = carry
                half = pl.ds(pl.multiple_of(c * (rc // 2), rc // 2), rc // 2)
                st = jnp.dot(_as_bf16(k_v[g, half, :]), _as_bf16(qm0[...]),
                             preferred_element_type=_f32)
                m_new = jnp.maximum(m, jnp.max(st, axis=0, keepdims=True))
                alpha = jnp.exp2(m - m_new)
                p = jnp.exp2(st - m_new)
                l = alpha * l + jnp.sum(p, axis=0, keepdims=True)
                vt = _as_bf16(vt_v[vrow, pl.ds(pl.multiple_of(c * rc, rc), rc)])
                acc = alpha * acc + jnp.dot(vt, p.astype(_bf16), preferred_element_type=_f32)
                return m_new, l, acc

            _, l, acc = jax.lax.fori_loop(
                0, S // rc, chunk,
                (jnp.full((1, _BQ), -jnp.inf, _f32), jnp.zeros((1, _BQ), _f32),
                 jnp.zeros((16, _BQ), _f32)))
            ot_v[vrow, pl.ds(pl.multiple_of(qb * _BQ, _BQ), _BQ)] = _as_u32((acc / l).astype(_bf16))

        jax.lax.fori_loop(0, nitems, item_body, None)

    c_o.wait()
    idx = idx_s[0]
    upd = upd_v[pl.ds(0, 1), :]

    def out_copy(b):
        return pltpu.make_async_copy(
            out_v.at[pl.ds(b * _TB, _TB), :], out_hbm.at[0, pl.ds(b * _TB, _TB), :], sem_o.at[b])

    for b in range(ntb):
        rows = pl.ds(b * _TB, _TB)
        ot = _as_bf16(ot_v[:, rows])
        a = jax.lax.dot_general(ot, wo_v[...], (((0,), (0,)), ((), ())),
                                preferred_element_type=_f32)
        xa = _rnd(x_v[rows, :].astype(_f32) + _rnd(a))
        tok = jax.lax.broadcasted_iota(jnp.int32, (_TB, D), 0) + b * _TB
        xn = xn_v[rows, :].astype(_f32)
        bb = jnp.where(tok == idx, _rnd(xn + upd), xn)
        out_v[rows, :] = (xa + bb).astype(_bf16)
        out_copy(b).start()
    for b in range(ntb):
        out_copy(b).wait()


@jax.jit
def pallas_parallel_sum__softmax_full_mha__moe_arch_mod__prompt_kernel(
    A_x: jax.Array,
    A_wqkv: jax.Array,
    A_wo: jax.Array,
    B_x: jax.Array,
    B_w_r: jax.Array,
    B_w_gate: jax.Array,
    B_w_up: jax.Array,
    B_w_down: jax.Array,
):
    del B_x
    B, S, D = A_x.shape
    F = B_w_gate.shape[1]
    assert B == 1 and D == _H * _DH and S % _BQ == 0 and S % _TB == 0
    ntb = S // _TB
    any_spec = pl.BlockSpec(memory_space=pl.ANY)
    u32 = jnp.uint32
    scratch = [
        pltpu.VMEM((S, D), _bf16),
        pltpu.VMEM((D, 3 * D), _bf16),
        pltpu.VMEM((D, D), _bf16),
        pltpu.VMEM((D,), _bf16),
        pltpu.VMEM((D, F), _bf16),
        pltpu.VMEM((D, F), _bf16),
        pltpu.VMEM((F, D), _bf16),
        pltpu.VMEM((S, D), _bf16),
        pltpu.VMEM((2 * D + 16, D), _bf16),
        pltpu.VMEM((D // 128, S // 2, 128), u32),
        pltpu.VMEM((D // 2, S), u32),
        pltpu.VMEM((D // 2, S), u32),
        pltpu.VMEM((8, S), _f32),
        pltpu.VMEM((S // 2, _BQ), u32),
        pltpu.VMEM((S // 2, _BQ), u32),
        pltpu.VMEM((64, _BQ), u32),
        pltpu.VMEM((64, _BQ), u32),
        pltpu.VMEM((D // 2, S), u32),
        pltpu.VMEM((8, _BQ), _f32),
        pltpu.VMEM((8, D), _f32),
        pltpu.SMEM((1,), jnp.int32),
        pltpu.VMEM((S, D), _bf16),
        pltpu.SemaphoreType.DMA((ntb,)),
        pltpu.SemaphoreType.DMA((6,)),
        pltpu.SemaphoreType.DMA((ntb,)),
    ]
    return pl.pallas_call(
        _kernel,
        in_specs=[any_spec] * 7,
        out_specs=any_spec,
        out_shape=jax.ShapeDtypeStruct((B, S, D), A_x.dtype),
        scratch_shapes=scratch,
        compiler_params=pltpu.CompilerParams(vmem_limit_bytes=96 * 1024 * 1024),
        name="fused_mha_mod_ffn",
    )(A_x, A_wqkv, A_wo, B_w_r, B_w_gate, B_w_up, B_w_down)
```

```python
import math

import jax
import jax.numpy as jnp
import jax.experimental.pallas as pl
import jax.experimental.pallas.tpu as pltpu

_H = 32
_DH = 16
_HG = 8
_BQ = 512
_R = 128
_UNROLL = 8
_TB = 256
_OB = 128
_EPS = 1e-5
_L_LO = 2.0 ** -80
_L_HI = 2.0 ** 90

_f32 = jnp.float32
_bf16 = jnp.bfloat16


def _as_bf16(u):
    return pltpu.bitcast(u, _bf16)


def _as_u32(x):
    return pltpu.bitcast(x, jnp.uint32)


def _rnd(x):
    return x.astype(_bf16).astype(_f32)


def _kernel(x_hbm, wqkv_hbm, wo_hbm, wr_hbm, wg_hbm, wu_hbm, wd_hbm, out_hbm,
            x_v, wqkv_v, wo_v, wr_v, wg_v, wu_v, wd_v,
            xn_v, wt_v, k_v, qt_v, vt_v, r_v, p0, p1, qm0, qm1, ot_v,
            upd_v, idx_s, out_v, sem_x, sem_w, sem_o):
    S, D = x_v.shape
    F = wg_v.shape[1]
    ntb = S // _TB
    nqb = S // _BQ
    nitems = _H * nqb
    nchunks = S // _R
    qscale = (_DH ** -0.5) * math.log2(math.e)

    def x_copy(b):
        return pltpu.make_async_copy(
            x_hbm.at[0, pl.ds(b * _TB, _TB), :], x_v.at[pl.ds(b * _TB, _TB), :], sem_x.at[b])

    def w_copy(i):
        cols = pl.ds(i * D, D)
        return pltpu.make_async_copy(wqkv_hbm.at[:, cols], wqkv_v.at[:, cols], sem_w.at[i])

    c_q, c_k, c_v = w_copy(0), w_copy(1), w_copy(2)
    c_r = pltpu.make_async_copy(wr_hbm, wr_v, sem_w.at[3])
    c_g = pltpu.make_async_copy(wg_hbm, wg_v, sem_w.at[4])
    c_u = pltpu.make_async_copy(wu_hbm, wu_v, sem_w.at[5])
    c_d = pltpu.make_async_copy(wd_hbm, wd_v, sem_w.at[6])
    c_o = pltpu.make_async_copy(wo_hbm, wo_v, sem_w.at[7])
    x_copy(0).start()
    c_k.start()
    x_copy(1).start()
    p1[...] = jnp.zeros(p1.shape, jnp.uint32)

    eps_b = _rnd(jnp.full((1, 1), _EPS, _f32))

    def layernorm(b):
        rows = pl.ds(b * _TB, _TB)
        xb = x_v[rows, :].astype(_f32)
        mean = jnp.sum(xb, axis=-1, keepdims=True) * (1.0 / D)
        var = jnp.sum(jnp.square(xb - mean), axis=-1, keepdims=True) * (1.0 / D)
        cen = _rnd(xb - _rnd(mean))
        den = _rnd(jnp.sqrt(_rnd(_rnd(var) + eps_b)))
        xn = (cen * (1.0 / den)).astype(_bf16)
        xn_v[rows, :] = xn
        return xn

    def proj_k(b, xn):
        kk = jnp.dot(xn, wqkv_v[:, pl.ds(D, D)], preferred_element_type=_f32).astype(_bf16)
        for g in range(D // 128):
            k_v[g, pl.ds(b * _TB // 2, _TB // 2), :] = _as_u32(kk[:, g * 128:(g + 1) * 128])

    def proj_qvr(b, xn):
        rows = pl.ds(b * _TB, _TB)
        tt = jax.lax.dot_general(wt_v[...], xn, (((1,), (1,)), ((), ())),
                                 preferred_element_type=_f32)
        qt_v[:, rows] = _as_u32((tt[:D] * qscale).astype(_bf16))
        vt_v[:, rows] = _as_u32(tt[D:2 * D].astype(_bf16))
        r_v[:, rows] = tt[2 * D:2 * D + 8]

    x_copy(0).wait()
    c_k.wait()
    x_copy(2).start()
    c_q.start()
    c_v.start()
    c_r.start()
    xns = {0: layernorm(0)}
    proj_k(0, xns[0])
    x_copy(1).wait()
    for b in range(3, ntb):
        x_copy(b).start()
    xns[1] = layernorm(1)
    proj_k(1, xns[1])
    x_copy(2).wait()
    c_q.wait()
    c_v.wait()
    c_r.wait()
    wt_v[pl.ds(0, D), :] = wqkv_v[:, pl.ds(0, D)].T
    wt_v[pl.ds(D, D), :] = wqkv_v[:, pl.ds(2 * D, D)].T
    wt_v[pl.ds(2 * D, 16), :] = jnp.broadcast_to(wr_v[...].reshape(1, D), (16, D))
    for b in range(ntb):
        if b == 1:
            for bb in range(3, ntb):
                x_copy(bb).wait()
            c_g.start()
            c_u.start()
            c_d.start()
            c_o.start()
        if b + 2 < ntb:
            xns[b + 2] = layernorm(b + 2)
        proj_qvr(b, xn_v[pl.ds(b * _TB, _TB), :])
        if b + 2 < ntb:
            proj_k(b + 2, xns[b + 2])

    r = _rnd(r_v[pl.ds(0, 1), :])
    rmax = jnp.max(r, axis=1, keepdims=True)
    pos = jax.lax.broadcasted_iota(jnp.int32, (1, S), 1)
    idx = jnp.min(jnp.where(r == rmax, pos, S - 1))
    idx_s[0] = idx
    base = pl.multiple_of((idx // 16) * 16, 16)
    grp = xn_v[pl.ds(base, 16), :].astype(_f32)
    sel = jax.lax.broadcasted_iota(jnp.int32, (16, D), 0) == (idx - base)
    x_sel = jnp.sum(jnp.where(sel, grp, 0.0), axis=0, keepdims=True)
    x_sel = jnp.broadcast_to(x_sel, (16, D)).astype(_bf16)
    c_g.wait()
    c_u.wait()
    c_d.wait()
    ga = _rnd(jnp.dot(x_sel, wg_v[...], preferred_element_type=_f32))
    ua = _rnd(jnp.dot(x_sel, wu_v[...], preferred_element_type=_f32))
    act = _rnd(ga * _rnd(jax.nn.sigmoid(ga)))
    hh = (act * ua).astype(_bf16)
    y = _rnd(jnp.dot(hh, wd_v[...], preferred_element_type=_f32))
    gate = _rnd(jax.nn.sigmoid(rmax))
    upd_v[...] = _rnd(y[:8] * gate)

    def split(item):
        item = jnp.clip(item, 0, nitems - 1)
        return item % _H, item // _H

    def prep(item, qm):
        h, qb = split(item)
        g = h // _HG
        q = qt_v[pl.ds(pl.multiple_of(g * 64, 64), 64), pl.ds(pl.multiple_of(qb * _BQ, _BQ), _BQ)]
        hrow = jax.lax.broadcasted_iota(jnp.int32, (64, _BQ), 0) // 8
        qm[...] = jnp.where(hrow == h % _HG, q, jnp.uint32(0))

    def step(item, do_a, pa, qm, qm_next, pb, lb, bad):
        g = split(item)[0] // _HG
        hb, qbb = split(item - 1)
        vrow = pl.ds(pl.multiple_of(hb * 8, 8), 8)
        l = jnp.zeros((8, _BQ), _f32)
        acc = jnp.zeros((16, _BQ), _f32)
        for c in range(nchunks):
            half = pl.ds(c * _R // 2, _R // 2)
            if do_a:
                st = jnp.dot(_as_bf16(k_v[g, half, :]), _as_bf16(qm[...]),
                             preferred_element_type=_f32)
                p = jnp.exp2(st)
                pa[half, :] = _as_u32(p.astype(_bf16))
                l = l + jnp.sum(p.reshape(_R // 8, 8, _BQ), axis=0)
                if c == 2:
                    prep(item + 1, qm_next)
            acc = acc + jnp.dot(_as_bf16(vt_v[vrow, pl.ds(c * _R, _R)]), _as_bf16(pb[half, :]),
                                preferred_element_type=_f32)
        o = acc / lb
        ot_v[vrow, pl.ds(pl.multiple_of(qbb * _BQ, _BQ), _BQ)] = _as_u32(o.astype(_bf16))
        ok = (lb >= _L_LO) & (lb <= _L_HI)
        fin = (jnp.abs(o[:8]) < jnp.inf) & (jnp.abs(o[8:]) < jnp.inf)
        bad = jnp.where(ok & fin, bad, 1.0)
        return jnp.sum(l, axis=0, keepdims=True), bad

    prep(0, qm0)

    def body(j, carry):
        l1, bad = carry
        for u in range(0, _UNROLL, 2):
            it = j * _UNROLL + u
            l0, bad = step(it, True, p0, qm0, qm1, p1, l1, bad)
            l1, bad = step(it + 1, True, p1, qm1, qm0, p0, l0, bad)
        return l1, bad

    l1, bad = jax.lax.fori_loop(
        0, nitems // _UNROLL, body,
        (jnp.ones((1, _BQ), _f32), jnp.zeros((8, _BQ), _f32)))
    _, bad = step(nitems, False, None, None, None, p1, l1, bad)

    @pl.when(jnp.max(bad) > 0.0)
    def _():
        rc = 512

        def item_body(item, _):
            h, qb = split(item)
            g = h // _HG
            prep(item, qm0)
            vrow = pl.ds(pl.multiple_of(h * 8, 8), 8)

            def chunk(c, carry):
                m, l, acc = carry
                half = pl.ds(pl.multiple_of(c * (rc // 2), rc // 2), rc // 2)
                st = jnp.dot(_as_bf16(k_v[g, half, :]), _as_bf16(qm0[...]),
                             preferred_element_type=_f32)
                m_new = jnp.maximum(m, jnp.max(st, axis=0, keepdims=True))
                alpha = jnp.exp2(m - m_new)
                p = jnp.exp2(st - m_new)
                l = alpha * l + jnp.sum(p, axis=0, keepdims=True)
                vt = _as_bf16(vt_v[vrow, pl.ds(pl.multiple_of(c * rc, rc), rc)])
                acc = alpha * acc + jnp.dot(vt, p.astype(_bf16), preferred_element_type=_f32)
                return m_new, l, acc

            _, l, acc = jax.lax.fori_loop(
                0, S // rc, chunk,
                (jnp.full((1, _BQ), -jnp.inf, _f32), jnp.zeros((1, _BQ), _f32),
                 jnp.zeros((16, _BQ), _f32)))
            ot_v[vrow, pl.ds(pl.multiple_of(qb * _BQ, _BQ), _BQ)] = _as_u32((acc / l).astype(_bf16))

        jax.lax.fori_loop(0, nitems, item_body, None)

    nob = S // _OB
    c_o.wait()
    idx = idx_s[0]
    upd = upd_v[pl.ds(0, 1), :]

    def out_copy(b):
        return pltpu.make_async_copy(
            out_v.at[pl.ds(b * _OB, _OB), :], out_hbm.at[0, pl.ds(b * _OB, _OB), :], sem_o.at[b])

    for b in range(nob):
        rows = pl.ds(b * _OB, _OB)
        ot = _as_bf16(ot_v[:, rows])
        a = jax.lax.dot_general(ot, wo_v[...], (((0,), (0,)), ((), ())),
                                preferred_element_type=_f32)
        xa = _rnd(x_v[rows, :].astype(_f32) + _rnd(a))
        tok = jax.lax.broadcasted_iota(jnp.int32, (_OB, D), 0) + b * _OB
        xn = xn_v[rows, :].astype(_f32)
        bb = jnp.where(tok == idx, _rnd(xn + upd), xn)
        out_v[rows, :] = (xa + bb).astype(_bf16)
        out_copy(b).start()
    for b in range(nob):
        out_copy(b).wait()


@jax.jit
def pallas_parallel_sum__softmax_full_mha__moe_arch_mod__prompt_kernel(
    A_x: jax.Array,
    A_wqkv: jax.Array,
    A_wo: jax.Array,
    B_x: jax.Array,
    B_w_r: jax.Array,
    B_w_gate: jax.Array,
    B_w_up: jax.Array,
    B_w_down: jax.Array,
):
    del B_x
    B, S, D = A_x.shape
    F = B_w_gate.shape[1]
    assert B == 1 and D == _H * _DH and S % _BQ == 0 and S % _TB == 0
    ntb = S // _TB
    any_spec = pl.BlockSpec(memory_space=pl.ANY)
    u32 = jnp.uint32
    scratch = [
        pltpu.VMEM((S, D), _bf16),
        pltpu.VMEM((D, 3 * D), _bf16),
        pltpu.VMEM((D, D), _bf16),
        pltpu.VMEM((D,), _bf16),
        pltpu.VMEM((D, F), _bf16),
        pltpu.VMEM((D, F), _bf16),
        pltpu.VMEM((F, D), _bf16),
        pltpu.VMEM((S, D), _bf16),
        pltpu.VMEM((2 * D + 16, D), _bf16),
        pltpu.VMEM((D // 128, S // 2, 128), u32),
        pltpu.VMEM((D // 2, S), u32),
        pltpu.VMEM((D // 2, S), u32),
        pltpu.VMEM((8, S), _f32),
        pltpu.VMEM((S // 2, _BQ), u32),
        pltpu.VMEM((S // 2, _BQ), u32),
        pltpu.VMEM((64, _BQ), u32),
        pltpu.VMEM((64, _BQ), u32),
        pltpu.VMEM((D // 2, S), u32),
        pltpu.VMEM((8, D), _f32),
        pltpu.SMEM((1,), jnp.int32),
        pltpu.VMEM((S, D), _bf16),
        pltpu.SemaphoreType.DMA((ntb,)),
        pltpu.SemaphoreType.DMA((8,)),
        pltpu.SemaphoreType.DMA((S // _OB,)),
    ]
    return pl.pallas_call(
        _kernel,
        in_specs=[any_spec] * 7,
        out_specs=any_spec,
        out_shape=jax.ShapeDtypeStruct((B, S, D), A_x.dtype),
        scratch_shapes=scratch,
        compiler_params=pltpu.CompilerParams(vmem_limit_bytes=96 * 1024 * 1024, flags={"XLA_TPU_EVENLY_DISTRIBUTE_CRITICAL_NODES": True}),
        name="fused_mha_mod_ffn",
    )(A_x, A_wqkv, A_wo, B_w_r, B_w_gate, B_w_up, B_w_down)
```
